```python
import jax
import jax.numpy as jnp

def _softmax(x, axis=-1):
    return jax.nn.softmax(x, axis=axis)
def _gelu(x):
    return jax.nn.gelu(x, approximate=True)
def _silu(x):
    return jax.nn.silu(x)
def _sigmoid(x):
    return jax.nn.sigmoid(x)
def _layernorm(x, axis=-1, eps=1e-5):
    m = jnp.mean(x, axis=axis, keepdims=True)
    v = jnp.var(x, axis=axis, keepdims=True)
    return (x - m) / jnp.sqrt(v + eps)
def _scatter_add(tgt, idx, src, axis=0):
    return tgt.at[idx].add(src)
def _segment_sum(src, seg, n):
    return jax.ops.segment_sum(src, seg, n)
class _Rng:
    def __init__(self, key):
        self._k = key
    def _next(self):
        self._k, sub = jax.random.split(self._k)
        return sub
    def normal(self, shape):
        return jax.random.normal(self._next(), shape, dtype=jnp.bfloat16)
    def randint(self, lo, hi, shape):
        return jax.random.randint(self._next(), shape, lo, hi, dtype=jnp.int32)
    def uniform(self, shape, lo=0.0, hi=1.0):
        return jax.random.uniform(self._next(), shape, jnp.bfloat16, lo, hi)
    def permutation(self, n):
        return jax.random.permutation(self._next(), n)


kernel_name = 'standalone__groupnorm__prompt'

def setup_inputs():
    _rng = _Rng(jax.random.key(int.from_bytes(__import__("os").urandom(4), "little")))
    _w = (lambda a: (lambda t: t.astype(jnp.bfloat16) if jnp.issubdtype(t.dtype, jnp.floating) else t)(jnp.asarray(a)))
    B = 2
    G = 32
    cpg = max(1, 1024 // G)
    C = G * cpg
    H, W = 32, 2048
    return {
        "x": _w((lambda *s: _rng.normal(s) * 0.05)(B, C, H, W)),
        "g": _w((lambda *s: _rng.normal(s) * 0.05)(C) + 1.0),
        "b": _w((lambda *s: _rng.normal(s) * 0.05)(C)),
    }

def reference(x, g, b):
    G = 32
    B, C, H, W = x.shape[0], x.shape[1], x.shape[2], x.shape[3]
    xr = x.reshape(B, G, C // G, H, W)
    mu = xr.mean(axis=(2, 3, 4), keepdims=True)
    var = ((xr - mu) ** 2).mean(axis=(2, 3, 4), keepdims=True)
    xn = (xr - mu) / jnp.sqrt(var + 1e-5)
    xn = xn.reshape(B, C, H, W)
    return xn * g[None, :, None, None] + b[None, :, None, None]
```

```python
import functools

import jax
import jax.numpy as jnp
from jax import lax
import jax.experimental.pallas as pl
import jax.experimental.pallas.tpu as pltpu

_G = 32
_EPS = 1e-5
_LANES = 128
_VREG_ROWS = 16

_SLOTS = 16
_STREAMS = 8
_AHEAD = 2
_READ_ROWS, _READ_TAIL = 128, 1
_WRITE_ROWS, _WRITE_TAIL = 32, 4
_NUM_ACC = 4


def _groupnorm_kernel(x_hbm, g_hbm, b_hbm, o_hbm, buf, gb_raw, g_tab, b_tab, rsem, wsem, gsem):
    ngroups, nstream, cps, ch_rows, _ = x_hbm.shape
    cpg = nstream * cps
    nphase = ngroups // _SLOTS
    inv_n = 1.0 / (cpg * ch_rows * _LANES)

    def start_copies(is_read, sems, rows, tail, grp, slot):
        pieces = ch_rows // rows

        def start(c, j, sem):
            r = pl.ds(j * rows, rows)
            if is_read:
                pltpu.make_async_copy(x_hbm.at[grp, :, c, r], buf.at[slot, :, c, r], sem).start()
            else:
                pltpu.make_async_copy(buf.at[slot, :, c, r], o_hbm.at[grp, :, c, r], sem).start()

        @pl.loop(0, cps - 1)
        def _(c):
            for j in range(pieces):
                start(c, j, sems.at[slot, 0])

        for j in range(pieces):
            start(cps - 1, j, sems.at[slot, int(j >= pieces - tail)])

    def wait(view, sem):
        pltpu.make_async_copy(view, view, sem).wait()

    def wait_head(sems, rows, tail, slot):
        wait(buf.at[slot, :, pl.ds(0, cps - 1)], sems.at[slot, 0])
        wait(buf.at[slot, :, cps - 1, pl.ds(0, ch_rows - rows * tail)], sems.at[slot, 0])

    def wait_tail(sems, rows, tail, slot):
        wait(buf.at[slot, :, cps - 1, pl.ds(ch_rows - rows * tail, rows * tail)], sems.at[slot, 1])

    read = (rsem, _READ_ROWS, _READ_TAIL)
    write = (wsem, _WRITE_ROWS, _WRITE_TAIL)
    start_read = functools.partial(start_copies, True, *read)
    start_write = functools.partial(start_copies, False, *write)

    tiles = [(c, pl.ds(r, _VREG_ROWS)) for c in range(cps) for r in range(0, ch_rows, _VREG_ROWS)]

    def group_mean(slot, fn):
        def body(s, accs):
            view = buf.at[slot, s]
            accs = list(accs)
            for t, (c, r) in enumerate(tiles):
                accs[t % _NUM_ACC] += fn(view[c, r, :].astype(jnp.float32))
            return tuple(accs)

        zero = jnp.zeros((_VREG_ROWS, _LANES), jnp.float32)
        total = functools.reduce(jnp.add, lax.fori_loop(0, nstream, body, (zero,) * _NUM_ACC))
        return jnp.sum(jnp.sum(total, axis=0, keepdims=True), axis=1, keepdims=True) * inv_n

    def normalize(grp, slot):
        mu = group_mean(slot, lambda v: v)
        var = group_mean(slot, lambda v: jnp.square(v - mu))
        rstd = 1.0 / jnp.sqrt(var + _EPS)
        ch0 = lax.rem(grp, _G) * cpg

        @pl.loop(0, nstream)
        def _(s):
            view = buf.at[slot, s]
            chans = [pl.ds(ch0 + s * cps + c, 1) for c in range(cps)]
            scale = [g_tab[ch, :] * rstd for ch in chans]
            shift = [b_tab[ch, :] for ch in chans]
            for c, r in tiles:
                v = view[c, r, :].astype(jnp.float32)
                view[c, r, :] = ((v - mu) * scale[c] + shift[c]).astype(buf.dtype)

    start_read(0, 0)
    params = [
        pltpu.make_async_copy(src, gb_raw.at[i], gsem.at[i]) for i, src in enumerate((g_hbm, b_hbm))
    ]
    for copy in params:
        copy.start()
    for i in range(1, _AHEAD):
        start_read(i, i)
    for i, tab in enumerate((g_tab, b_tab)):
        params[i].wait()
        v = gb_raw[i].astype(jnp.float32)
        for r in range(v.shape[0]):
            tab[pl.ds(r * _LANES, _LANES), :] = jnp.broadcast_to(v[r : r + 1, :], (_LANES, _LANES)).T

    @pl.loop(0, nphase)
    def _(p):
        g0 = p * _SLOTS

        @pl.loop(0, _SLOTS)
        def _(k):
            @pl.when(k + _AHEAD < _SLOTS)
            def _():
                start_read(g0 + k + _AHEAD, k + _AHEAD)

            wait_head(*read, k)

            @pl.when(k == _SLOTS - 1)
            def _():
                pl.loop(0, _AHEAD)(lambda i: start_write(g0 + i, i))

            wait_tail(*read, k)
            normalize(g0 + k, k)

        @pl.loop(0, _SLOTS)
        def _(k):
            @pl.when(k + _AHEAD < _SLOTS)
            def _():
                start_write(g0 + k + _AHEAD, k + _AHEAD)

            wait_head(*write, k)

            @pl.when(jnp.logical_and(k == _SLOTS - 1, p + 1 < nphase))
            def _():
                pl.loop(0, _AHEAD)(lambda i: start_read(g0 + _SLOTS + i, i))

            wait_tail(*write, k)


@jax.jit
def pallas_standalone__groupnorm__prompt_kernel(
    x: jax.Array,
    g: jax.Array,
    b: jax.Array,
):
    B, C, H, W = x.shape
    cpg = C // _G
    shape = (B * _G, _STREAMS, cpg // _STREAMS, H * W // _LANES, _LANES)
    xt = x.reshape(B * C, H // 8, 8, W // _LANES, _LANES).transpose(0, 1, 3, 2, 4).reshape(shape)
    group_bytes = cpg * H * W * x.dtype.itemsize
    out = pl.pallas_call(
        _groupnorm_kernel,
        in_specs=[pl.BlockSpec(memory_space=pl.ANY)] * 3,
        out_specs=pl.BlockSpec(memory_space=pl.ANY),
        out_shape=jax.ShapeDtypeStruct(shape, x.dtype),
        scratch_shapes=[
            pltpu.VMEM((_SLOTS,) + shape[1:], x.dtype),
            pltpu.VMEM((2, C // _LANES, _LANES), g.dtype),
            pltpu.VMEM((C, _LANES), jnp.float32),
            pltpu.VMEM((C, _LANES), jnp.float32),
            pltpu.SemaphoreType.DMA((_SLOTS, 2)),
            pltpu.SemaphoreType.DMA((_SLOTS, 2)),
            pltpu.SemaphoreType.DMA((2,)),
        ],
        compiler_params=pltpu.CompilerParams(
            vmem_limit_bytes=_SLOTS * group_bytes + 8 * 1024 * 1024,
        ),
    )(xt, g.reshape(C // _LANES, _LANES), b.reshape(C // _LANES, _LANES))
    return out.reshape(B * C, H // 8, W // _LANES, 8, _LANES).transpose(0, 1, 3, 2, 4).reshape(x.shape)
```

```python
import functools

import jax
import jax.numpy as jnp
from jax import lax
import jax.experimental.pallas as pl
import jax.experimental.pallas.tpu as pltpu

_G = 32
_EPS = 1e-5
_LANES = 128
_VREG_ROWS = 16
_NUM_ACC = 4

_PHASE = 22
_SLOTS = _PHASE + 1
_STREAMS = 8
_PIECE = 32
_DEPTH = 16
_LEAD = 8
_LAG = 4
_READ_TAIL = 7
_WRITE_TAIL = 2
_HIGH, _LOW = 0, 1


def _groupnorm_kernel(
    x_hbm, g_hbm, b_hbm, o_hbm, buf, gb_raw, g_tab, b_tab, low_sem, high_sem, write_sem, once_sem
):
    ngroups, nstream, cps, ch_rows, _ = x_hbm.shape
    cpg = nstream * cps
    pieces = ch_rows // _PIECE
    strips = cps * pieces

    def wrap(slot):
        return jnp.where(slot >= _SLOTS, slot - _SLOTS, slot)

    def split_tail(ref, tail):
        cut = ch_rows - tail * _PIECE
        return (
            ref.at[:, pl.ds(0, cps - 1)],
            ref.at[:, cps - 1, pl.ds(0, cut)],
            ref.at[:, cps - 1, pl.ds(cut, ch_rows - cut)],
        )

    def read_copy(grp0, slot0, ways, t, high):
        q = lax.div(t, ways)
        k = lax.div(q, strips) * ways + lax.rem(t, ways)
        j = lax.rem(q, strips)
        c = lax.div(j, pieces)
        r = pl.ds(pl.multiple_of(lax.rem(j, pieces) * _PIECE, _PIECE), _PIECE)
        s = pl.ds(nstream - 1, 1) if high else pl.ds(0, nstream - 1)
        sem = (high_sem if high else low_sem).at[lax.rem(t, _DEPTH)]
        return pltpu.make_async_copy(x_hbm.at[grp0 + k, s, c, r], buf.at[wrap(slot0 + k), s, c, r], sem)

    def start_reads(*run):
        @pl.loop(0, _LEAD)
        def _(t):
            read_copy(*run, t, False).start(priority=_LOW)
            read_copy(*run, t, True).start(priority=_HIGH)

        @pl.loop(_LEAD, _DEPTH)
        def _(t):
            read_copy(*run, t, False).start(priority=_LOW)

    def finish_reads(run, total, tail, on_tail):
        @pl.loop(0, total)
        def _(t):
            read_copy(*run, t, False).wait()

            @pl.when(t >= _LAG)
            def _():
                read_copy(*run, t - _LAG, True).wait()

            @pl.when(t + _LEAD < total)
            def _():
                read_copy(*run, t + _LEAD, True).start(priority=_HIGH)

            @pl.when(t + _DEPTH < total)
            def _():
                read_copy(*run, t + _DEPTH, False).start(priority=_LOW)

            pl.when(t == total - 1 - tail)(on_tail)

        @pl.loop(total - _LAG, total)
        def _(t):
            read_copy(*run, t, True).wait()

    def start_write(grp, slot):
        def start(c, j, part):
            r = pl.ds(j * _PIECE, _PIECE)
            sem = write_sem.at[lax.rem(grp, 2), part]
            pltpu.make_async_copy(buf.at[slot, :, c, r], o_hbm.at[grp, :, c, r], sem).start()

        @pl.loop(0, cps - 1)
        def _(c):
            for j in range(pieces):
                start(c, j, 0)

        for j in range(pieces):
            start(cps - 1, j, 1 if j < pieces - _WRITE_TAIL else 2)

    def finish_write(grp, slot, on_tail):
        src, dst = split_tail(buf.at[slot], _WRITE_TAIL), split_tail(o_hbm.at[grp], _WRITE_TAIL)
        for part in range(3):
            if part == 2:
                on_tail()
            pltpu.make_async_copy(src[part], dst[part], write_sem.at[lax.rem(grp, 2), part]).wait()

    inv_n = 1.0 / (cpg * ch_rows * _LANES)
    tiles = [(c, pl.ds(r, _VREG_ROWS)) for c in range(cps) for r in range(0, ch_rows, _VREG_ROWS)]

    def group_mean(slot, fn):
        def body(s, accs):
            view = buf.at[slot, s]
            accs = list(accs)
            for i, (c, r) in enumerate(tiles):
                accs[i % _NUM_ACC] += fn(view[c, r, :].astype(jnp.float32))
            return tuple(accs)

        zero = jnp.zeros((_VREG_ROWS, _LANES), jnp.float32)
        total = functools.reduce(jnp.add, lax.fori_loop(0, nstream, body, (zero,) * _NUM_ACC))
        return jnp.sum(jnp.sum(total, axis=0, keepdims=True), axis=1, keepdims=True) * inv_n

    def normalize(grp, slot):
        mu = group_mean(slot, lambda v: v)
        var = group_mean(slot, lambda v: jnp.square(v - mu))
        rstd = 1.0 / jnp.sqrt(var + _EPS)
        ch0 = lax.rem(grp, _G) * cpg

        @pl.loop(0, nstream)
        def _(s):
            view = buf.at[slot, s]
            chans = [pl.ds(ch0 + s * cps + c, 1) for c in range(cps)]
            scale = [g_tab[ch, :] * rstd for ch in chans]
            shift = [b_tab[ch, :] for ch in chans]
            for c, r in tiles:
                v = view[c, r, :].astype(jnp.float32)
                view[c, r, :] = ((v - mu) * scale[c] + shift[c]).astype(buf.dtype)

    start_reads(0, 0, 1)
    params = [
        pltpu.make_async_copy(src, gb_raw.at[i], once_sem.at[i]) for i, src in enumerate((g_hbm, b_hbm))
    ]
    for copy in params:
        copy.start()
    second = [
        pltpu.make_async_copy(src, dst, once_sem.at[2 + i])
        for i, (src, dst) in enumerate(
            zip(split_tail(x_hbm.at[1], _READ_TAIL), split_tail(buf.at[1], _READ_TAIL))
        )
    ]

    def start_second():
        for copy in second:
            copy.start(priority=_LOW)

    finish_reads((0, 0, 1), strips, _DEPTH - 1, start_second)
    for i, tab in enumerate((g_tab, b_tab)):
        params[i].wait()
        v = gb_raw[i].astype(jnp.float32)
        for r in range(v.shape[0]):
            tab[pl.ds(r * _LANES, _LANES), :] = jnp.broadcast_to(v[r : r + 1, :], (_LANES, _LANES)).T
    normalize(0, 0)
    second[0].wait()
    second[1].wait()
    start_reads(2, 2, 2)
    second[2].wait()

    def phase(p, first_slot):
        read_lo, read_hi = jnp.maximum(p * _PHASE, 2), jnp.minimum((p + 1) * _PHASE, ngroups)
        write_lo = jnp.maximum(p * _PHASE - 1, 0)
        write_hi = jnp.where(read_hi == ngroups, ngroups, read_hi - 1)
        finish_reads(
            (read_lo, wrap(first_slot + read_lo - write_lo), 2),
            (read_hi - read_lo) * strips,
            _READ_TAIL,
            lambda: start_write(write_lo, first_slot),
        )

        def write_step(j, slot):
            nxt = wrap(slot + 1)
            pl.when(j + 1 < read_hi)(lambda: normalize(j + 1, nxt))
            pl.when(j + 1 < write_hi)(lambda: start_write(j + 1, nxt))
            more = jnp.logical_and(j + 1 == write_hi, read_hi < ngroups)
            finish_write(j, slot, lambda: pl.when(more)(lambda: start_reads(read_hi, wrap(nxt + 1), 2)))
            return nxt

        return lax.fori_loop(write_lo, write_hi, write_step, first_slot)

    lax.fori_loop(0, pl.cdiv(ngroups, _PHASE), phase, 0)


@jax.jit
def pallas_standalone__groupnorm__prompt_kernel(
    x: jax.Array,
    g: jax.Array,
    b: jax.Array,
):
    B, C, H, W = x.shape
    cpg = C // _G
    shape = (B * _G, _STREAMS, cpg // _STREAMS, H * W // _LANES, _LANES)
    xt = x.reshape(B * C, H // 8, 8, W // _LANES, _LANES).transpose(0, 1, 3, 2, 4).reshape(shape)
    group_bytes = cpg * H * W * x.dtype.itemsize
    out = pl.pallas_call(
        _groupnorm_kernel,
        in_specs=[pl.BlockSpec(memory_space=pl.ANY)] * 3,
        out_specs=pl.BlockSpec(memory_space=pl.ANY),
        out_shape=jax.ShapeDtypeStruct(shape, x.dtype),
        scratch_shapes=[
            pltpu.VMEM((_SLOTS,) + shape[1:], x.dtype),
            pltpu.VMEM((2, C // _LANES, _LANES), g.dtype),
            pltpu.VMEM((C, _LANES), jnp.float32),
            pltpu.VMEM((C, _LANES), jnp.float32),
            pltpu.SemaphoreType.DMA((_DEPTH,)),
            pltpu.SemaphoreType.DMA((_DEPTH,)),
            pltpu.SemaphoreType.DMA((2, 3)),
            pltpu.SemaphoreType.DMA((5,)),
        ],
        compiler_params=pltpu.CompilerParams(
            vmem_limit_bytes=(_SLOTS + 1) * group_bytes,
            disable_bounds_checks=True,
        ),
    )(xt, g.reshape(C // _LANES, _LANES), b.reshape(C // _LANES, _LANES))
    return out.reshape(B * C, H // 8, W // _LANES, 8, _LANES).transpose(0, 1, 3, 2, 4).reshape(x.shape)
```

```python
import functools

import jax
import jax.numpy as jnp
from jax import lax
import jax.experimental.pallas as pl
import jax.experimental.pallas.tpu as pltpu

_G = 32
_EPS = 1e-5
_LANES = 128
_VREG_ROWS = 16
_NUM_ACC = 2

_PAIR = 2
_WAYS = 4
_SLOTS = 12
_STREAMS = 4
_PIECE = 64
_DEPTH = 16
_LEAD = 8
_LAG = 4
_READ_TAIL = 7
_WRITE_TAIL = 1
_HIGH, _LOW = 0, 1
_CHUNK = 1024
_PACED_CHUNK = 256


def _div(a, n):
    assert n & (n - 1) == 0
    return a >> (n.bit_length() - 1)


def _rem(a, n):
    assert n & (n - 1) == 0
    return a & (n - 1)


def _groupnorm_kernel(
    x_hbm, g_hbm, b_hbm, o_hbm, buf, gb_raw, gb_f32, gb_smem, low_sem, high_sem, write_sem, gb_sem
):
    npairs, _, cps, ch_rows, _ = x_hbm.shape
    cpg = _STREAMS * cps
    pieces = ch_rows // _PIECE
    strips = cps * pieces
    inv_n = 1.0 / (cpg * ch_rows * _LANES)

    def read_copy(base, t, high):
        q = _div(t, _WAYS)
        grp = _div(q, strips) * _WAYS + _rem(t, _WAYS)
        j = _rem(q, strips)
        s0 = _rem(grp, _PAIR) * _STREAMS
        where = (
            pl.ds(s0 + _STREAMS - 1, 1) if high else pl.ds(s0, _STREAMS - 1),
            _div(j, pieces),
            pl.ds(pl.multiple_of(_rem(j, pieces) * _PIECE, _PIECE), _PIECE),
        )
        slot = _div(grp, _PAIR)
        sem = (high_sem if high else low_sem).at[_rem(t, _DEPTH)]
        return pltpu.make_async_copy(x_hbm.at[base + slot, *where], buf.at[slot, *where], sem)

    def start_reads(base):
        @pl.loop(0, _LEAD)
        def _(t):
            read_copy(base, t, False).start(priority=_LOW)
            read_copy(base, t, True).start(priority=_HIGH)

        @pl.loop(_LEAD, _DEPTH)
        def _(t):
            read_copy(base, t, False).start(priority=_LOW)

    def read_step(base, t, start_high=True, start_low=True, wait_high=True):
        read_copy(base, t, False).wait()
        if start_high:
            read_copy(base, t + _LEAD, True).start(priority=_HIGH)
        if start_low:
            read_copy(base, t + _DEPTH, False).start(priority=_LOW)
        if wait_high:
            read_copy(base, t - _LAG, True).wait()

    def start_write(base, slot):
        def start(c, j, part):
            where = (slice(None), c, pl.ds(j * _PIECE, _PIECE))
            sem = write_sem.at[_rem(slot, 2), part]
            pltpu.make_async_copy(buf.at[slot, *where], o_hbm.at[base + slot, *where], sem).start()

        @pl.loop(0, cps - 1)
        def _(c):
            for j in range(pieces):
                start(c, j, 0)

        for j in range(pieces):
            start(cps - 1, j, 1 if j < pieces - _WRITE_TAIL else 2)

    def wait_write(base, slot, part):
        cut = ch_rows - _WRITE_TAIL * _PIECE
        where = (
            (slice(None), pl.ds(0, cps - 1)),
            (slice(None), cps - 1, pl.ds(0, cut)),
            (slice(None), cps - 1, pl.ds(cut, ch_rows - cut)),
        )[part]
        sem = write_sem.at[_rem(slot, 2), part]
        pltpu.make_async_copy(buf.at[slot, *where], o_hbm.at[base + slot, *where], sem).wait()

    def normalize(base, slot, chunk, tick=lambda i: None):
        nch, parts = max(chunk // ch_rows, 1), max(ch_rows // chunk, 1)
        rows = ch_rows // parts
        nchunk = cpg // nch * parts
        tiles = [(c, pl.ds(r, _VREG_ROWS)) for c in range(nch) for r in range(0, rows, _VREG_ROWS)]

        @pl.loop(0, _PAIR)
        def _(h):
            def next_chunk(sweep, i):
                tick((h * 3 + sweep) * nchunk + i)
                ch = _div(i, parts) * nch
                r = pl.ds(pl.multiple_of(_rem(i, parts) * rows, rows), rows)
                return ch, buf.at[slot, h * _STREAMS + _div(ch, cps), pl.ds(_rem(ch, cps), nch), r]

            def group_mean(sweep, fn):
                def body(i, accs):
                    _, view = next_chunk(sweep, i)
                    accs = list(accs)
                    for n, (c, r) in enumerate(tiles):
                        accs[n % _NUM_ACC] += fn(view[c, r, :].astype(jnp.float32))
                    return tuple(accs)

                zero = jnp.zeros((_VREG_ROWS, _LANES), jnp.float32)
                total = functools.reduce(jnp.add, lax.fori_loop(0, nchunk, body, (zero,) * _NUM_ACC))
                return jnp.sum(jnp.sum(total, axis=0, keepdims=True), axis=1, keepdims=True) * inv_n

            mu = group_mean(0, lambda v: v)
            var = group_mean(1, lambda v: jnp.square(v - mu))
            rstd = 1.0 / jnp.sqrt(var + _EPS)
            ch0 = _rem((base + slot) * _PAIR + h, _G) * cpg

            @pl.loop(0, nchunk)
            def _(i):
                ch, view = next_chunk(2, i)
                row, col = _div(ch0 + ch, _LANES), _rem(ch0 + ch, _LANES)
                scale = [gb_smem[0, row, col + c] * rstd for c in range(nch)]
                shift = [gb_smem[1, row, col + c] for c in range(nch)]
                for c, r in tiles:
                    v = view[c, r, :].astype(jnp.float32)
                    view[c, r, :] = ((v - mu) * scale[c] + shift[c]).astype(buf.dtype)

        return _PAIR * 3 * nchunk

    params = [
        pltpu.make_async_copy(src, gb_raw.at[i], gb_sem.at[i]) for i, src in enumerate((g_hbm, b_hbm))
    ]
    for copy in params:
        copy.start()
    start_reads(0)
    for copy in params:
        copy.wait()
    gb_f32[...] = gb_raw[...].astype(jnp.float32)
    pltpu.sync_copy(gb_f32, gb_smem)

    @pl.loop(0, pl.cdiv(npairs, _SLOTS))
    def _(phase):
        base = phase * _SLOTS
        count = jnp.minimum(_SLOTS, npairs - base)
        total = count * _PAIR * strips
        step = functools.partial(read_step, base)

        arrived = _WAYS * strips + _LAG
        pl.loop(0, _LAG)(functools.partial(step, wait_high=False))
        pl.loop(_LAG, arrived)(step)
        done = arrived + normalize(base, 0, _PACED_CHUNK, lambda i: step(arrived + i))
        assert done + _DEPTH <= (npairs % _SLOTS or _SLOTS) * _PAIR * strips
        pl.loop(done, total - _DEPTH)(step)
        pl.loop(total - _DEPTH, total - _LEAD)(functools.partial(step, start_low=False))

        @pl.loop(total - _LEAD, total)
        def _(t):
            step(t, start_high=False, start_low=False)
            pl.when(t == total - 1 - _READ_TAIL)(lambda: start_write(base, 0))

        pl.loop(total - _LAG, total)(lambda t: read_copy(base, t, True).wait())

        @pl.loop(0, count)
        def _(slot):
            @pl.when(slot + 1 < count)
            def _():
                normalize(base, slot + 1, _CHUNK)
                start_write(base, slot + 1)

            wait_write(base, slot, 0)
            wait_write(base, slot, 1)
            more = jnp.logical_and(slot + 1 == count, base + count < npairs)
            pl.when(more)(lambda: start_reads(base + count))
            wait_write(base, slot, 2)


@jax.jit
def pallas_standalone__groupnorm__prompt_kernel(
    x: jax.Array,
    g: jax.Array,
    b: jax.Array,
):
    B, C, H, W = x.shape
    cpg = C // _G
    shape = (B * _G // _PAIR, _PAIR * _STREAMS, cpg // _STREAMS, H * W // _LANES, _LANES)
    xt = x.reshape(B * C, H // 8, 8, W // _LANES, _LANES).transpose(0, 1, 3, 2, 4).reshape(shape)
    gb_shape = (C // _LANES, _LANES)
    pair_bytes = _PAIR * cpg * H * W * x.dtype.itemsize
    out = pl.pallas_call(
        _groupnorm_kernel,
        in_specs=[pl.BlockSpec(memory_space=pl.ANY)] * 3,
        out_specs=pl.BlockSpec(memory_space=pl.ANY),
        out_shape=jax.ShapeDtypeStruct(shape, x.dtype),
        scratch_shapes=[
            pltpu.VMEM((_SLOTS, *shape[1:]), x.dtype),
            pltpu.VMEM((2, *gb_shape), g.dtype),
            pltpu.VMEM((2, *gb_shape), jnp.float32),
            pltpu.SMEM((2, *gb_shape), jnp.float32),
            pltpu.SemaphoreType.DMA((_DEPTH,)),
            pltpu.SemaphoreType.DMA((_DEPTH,)),
            pltpu.SemaphoreType.DMA((2, 3)),
            pltpu.SemaphoreType.DMA((2,)),
        ],
        compiler_params=pltpu.CompilerParams(
            vmem_limit_bytes=_SLOTS * pair_bytes + 4 * 1024 * 1024,
            disable_bounds_checks=True,
            disable_semaphore_checks=True,
        ),
    )(xt, g.reshape(gb_shape), b.reshape(gb_shape))
    return out.reshape(B * C, H // 8, W // _LANES, 8, _LANES).transpose(0, 1, 3, 2, 4).reshape(x.shape)
```

```python
import functools

import jax
import jax.numpy as jnp
from jax import lax
import jax.experimental.pallas as pl
import jax.experimental.pallas.tpu as pltpu

_G = 32
_EPS = 1e-5
_LANES = 128
_VREG_ROWS = 16
_NUM_ACC = 2

_PHASE = 24
_STREAMS = 4
_PIECE = 64
_WAYS = 4
_SWEEP = 6
_DEPTH = 16
_LEAD = 8
_LAG = 4
_READ_TAIL = 7
_WRITE_TAIL = 1
_HIGH, _LOW = 0, 1
_CHUNK = 1024
_PACED_CHUNK = 256


def _div(a, n):
    assert n & (n - 1) == 0
    return a >> (n.bit_length() - 1)


def _rem(a, n):
    assert n & (n - 1) == 0
    return a & (n - 1)


def _groupnorm_kernel(
    x_hbm, g_hbm, b_hbm, o_hbm, buf, gb_raw, gb_f32, gb_smem, low_sem, high_sem, write_sem, gb_sem
):
    nstreams, cps, ch_rows, _ = x_hbm.shape
    ngroups = nstreams // _STREAMS
    cpg = _STREAMS * cps
    pieces = ch_rows // _PIECE
    strips = cps * pieces
    inv_n = 1.0 / (cpg * ch_rows * _LANES)

    def locate(base, first, count, *where):
        return (pl.ds(base * _STREAMS + first, count), *where), (pl.ds(first, count), *where)

    def read_copy(base, t, high):
        q = _div(t, _WAYS)
        first = (_div(q, strips) * _WAYS + _rem(t, _WAYS)) * _STREAMS
        j = _rem(q, strips)
        hbm, vmem = locate(
            base,
            *((first + _STREAMS - 1, 1) if high else (first, _STREAMS - 1)),
            _div(j, pieces),
            pl.ds(pl.multiple_of(_rem(j, pieces) * _PIECE, _PIECE), _PIECE),
        )
        sem = (high_sem if high else low_sem).at[_rem(t, _DEPTH)]
        return pltpu.make_async_copy(x_hbm.at[hbm], buf.at[vmem], sem)

    def start_reads(base):
        @pl.loop(0, _LEAD)
        def _(t):
            read_copy(base, t, False).start(priority=_LOW)
            read_copy(base, t, True).start(priority=_HIGH)

        @pl.loop(_LEAD, _DEPTH)
        def _(t):
            read_copy(base, t, False).start(priority=_LOW)

    def read_step(base, t, start_high=True, start_low=True, wait_high=True):
        read_copy(base, t, False).wait()
        if start_high:
            read_copy(base, t + _LEAD, True).start(priority=_HIGH)
        if start_low:
            read_copy(base, t + _DEPTH, False).start(priority=_LOW)
        if wait_high:
            read_copy(base, t - _LAG, True).wait()

    def write_copy(base, sweep, count, part, *where):
        hbm, vmem = locate(base, sweep * _SWEEP, count, *where)
        return pltpu.make_async_copy(buf.at[vmem], o_hbm.at[hbm], write_sem.at[_rem(sweep, 4), part])

    def start_sweep(base, sweep, count=_SWEEP):
        @pl.loop(0, cps - 1)
        def _(c):
            for j in range(pieces):
                write_copy(base, sweep, count, 0, c, pl.ds(j * _PIECE, _PIECE)).start()

        for j in range(pieces):
            part = 1 if j < pieces - _WRITE_TAIL else 2
            write_copy(base, sweep, count, part, cps - 1, pl.ds(j * _PIECE, _PIECE)).start()

    def finish_sweep(base, sweep, count=_SWEEP, before_tail=lambda: None):
        cut = ch_rows - _WRITE_TAIL * _PIECE
        write_copy(base, sweep, count, 0, pl.ds(0, cps - 1)).wait()
        write_copy(base, sweep, count, 1, cps - 1, pl.ds(0, cut)).wait()
        before_tail()
        write_copy(base, sweep, count, 2, cps - 1, pl.ds(cut, ch_rows - cut)).wait()

    def normalize(base, lo, hi, chunk, tick=lambda i: None):
        nch, parts = max(chunk // ch_rows, 1), max(ch_rows // chunk, 1)
        rows = ch_rows // parts
        nchunk = cpg // nch * parts
        tiles = [(c, pl.ds(r, _VREG_ROWS)) for c in range(nch) for r in range(0, rows, _VREG_ROWS)]

        @pl.loop(lo, hi)
        def _(grp):
            def next_chunk(stage, i):
                tick((grp * 3 + stage) * nchunk + i)
                ch = _div(i, parts) * nch
                r = pl.ds(pl.multiple_of(_rem(i, parts) * rows, rows), rows)
                return ch, buf.at[grp * _STREAMS + _div(ch, cps), pl.ds(_rem(ch, cps), nch), r]

            def group_mean(stage, fn):
                def body(i, accs):
                    _, view = next_chunk(stage, i)
                    accs = list(accs)
                    for n, (c, r) in enumerate(tiles):
                        accs[n % _NUM_ACC] += fn(view[c, r, :].astype(jnp.float32))
                    return tuple(accs)

                zero = jnp.zeros((_VREG_ROWS, _LANES), jnp.float32)
                total = functools.reduce(jnp.add, lax.fori_loop(0, nchunk, body, (zero,) * _NUM_ACC))
                return jnp.sum(jnp.sum(total, axis=0, keepdims=True), axis=1, keepdims=True) * inv_n

            mu = group_mean(0, lambda v: v)
            var = group_mean(1, lambda v: jnp.square(v - mu))
            rstd = 1.0 / jnp.sqrt(var + _EPS)
            ch0 = _rem(base + grp, _G) * cpg

            @pl.loop(0, nchunk)
            def _(i):
                ch, view = next_chunk(2, i)
                row, col = _div(ch0 + ch, _LANES), _rem(ch0 + ch, _LANES)
                scale = [gb_smem[0, row, col + c] * rstd for c in range(nch)]
                shift = [gb_smem[1, row, col + c] for c in range(nch)]
                for c, r in tiles:
                    v = view[c, r, :].astype(jnp.float32)
                    view[c, r, :] = ((v - mu) * scale[c] + shift[c]).astype(buf.dtype)

        return 3 * nchunk

    params = [
        pltpu.make_async_copy(src, gb_raw.at[i], gb_sem.at[i]) for i, src in enumerate((g_hbm, b_hbm))
    ]
    for copy in params:
        copy.start()
    start_reads(0)
    for copy in params:
        copy.wait()
    gb_f32[...] = gb_raw[...].astype(jnp.float32)
    pltpu.sync_copy(gb_f32, gb_smem)

    last_count = ngroups % _PHASE or _PHASE
    last_sweeps, spare = divmod(last_count * _STREAMS, _SWEEP)
    assert _PHASE * _STREAMS % _SWEEP == 0 and _PHASE % _WAYS == 0 and last_count % _WAYS == 0

    def groups_under(sweeps):
        return _div(sweeps * _SWEEP + _STREAMS - 1, _STREAMS)

    @pl.loop(0, pl.cdiv(ngroups, _PHASE))
    def _(phase):
        base = phase * _PHASE
        count = jnp.minimum(_PHASE, ngroups - base)
        more = base + count < ngroups
        total = count * strips
        step = functools.partial(read_step, base)

        arrived = _WAYS * strips + _LAG
        pl.loop(0, _LAG)(functools.partial(step, wait_high=False))
        pl.loop(_LAG, arrived)(step)
        ticks = normalize(base, 0, groups_under(1), _PACED_CHUNK, lambda i: step(arrived + i))
        done = arrived + groups_under(1) * ticks
        assert groups_under(1) <= _WAYS and done + _DEPTH <= last_count * strips
        pl.loop(done, total - _DEPTH)(step)
        pl.loop(total - _DEPTH, total - _LEAD)(functools.partial(step, start_low=False))

        @pl.loop(total - _LEAD, total)
        def _(t):
            step(t, start_high=False, start_low=False)
            pl.when(t == total - 1 - _READ_TAIL)(lambda: start_sweep(base, 0))

        pl.loop(total - _LAG, total)(lambda t: read_copy(base, t, True).wait())

        sweeps = jnp.where(more, _PHASE * _STREAMS // _SWEEP, last_sweeps)

        @pl.loop(1, sweeps + 1)
        def _(w):
            normalize(base, groups_under(w), jnp.minimum(groups_under(w + 1), count), _CHUNK)
            pl.when(w < sweeps)(lambda: start_sweep(base, w))
            pl.when(w >= 2)(lambda: finish_sweep(base, w - 2))

        @pl.when(more)
        def _():
            finish_sweep(base, sweeps - 1, before_tail=lambda: start_reads(base + count))

    if spare:
        start_sweep(ngroups - last_count, last_sweeps, spare)
    finish_sweep(ngroups - last_count, last_sweeps - 1)
    if spare:
        finish_sweep(ngroups - last_count, last_sweeps, spare)


@jax.jit
def pallas_standalone__groupnorm__prompt_kernel(
    x: jax.Array,
    g: jax.Array,
    b: jax.Array,
):
    B, C, H, W = x.shape
    cpg = C // _G
    shape = (B * _G * _STREAMS, cpg // _STREAMS, H * W // _LANES, _LANES)
    xt = x.reshape(B * C, H // 8, 8, W // _LANES, _LANES).transpose(0, 1, 3, 2, 4).reshape(shape)
    gb_shape = (C // _LANES, _LANES)
    group_bytes = cpg * H * W * x.dtype.itemsize
    out = pl.pallas_call(
        _groupnorm_kernel,
        in_specs=[pl.BlockSpec(memory_space=pl.ANY)] * 3,
        out_specs=pl.BlockSpec(memory_space=pl.ANY),
        out_shape=jax.ShapeDtypeStruct(shape, x.dtype),
        scratch_shapes=[
            pltpu.VMEM((_PHASE * _STREAMS, *shape[1:]), x.dtype),
            pltpu.VMEM((2, *gb_shape), g.dtype),
            pltpu.VMEM((2, *gb_shape), jnp.float32),
            pltpu.SMEM((2, *gb_shape), jnp.float32),
            pltpu.SemaphoreType.DMA((_DEPTH,)),
            pltpu.SemaphoreType.DMA((_DEPTH,)),
            pltpu.SemaphoreType.DMA((4, 3)),
            pltpu.SemaphoreType.DMA((2,)),
        ],
        compiler_params=pltpu.CompilerParams(
            vmem_limit_bytes=_PHASE * group_bytes + 4 * 1024 * 1024,
            disable_bounds_checks=True,
            disable_semaphore_checks=True,
        ),
    )(xt, g.reshape(gb_shape), b.reshape(gb_shape))
    return out.reshape(B * C, H // 8, W // _LANES, 8, _LANES).transpose(0, 1, 3, 2, 4).reshape(x.shape)
```
